```python
import os as _os
_os.environ.setdefault("JAX_PLATFORMS", "cpu")
import jax
import jax.numpy as jnp

def _softmax(x, axis=-1):
    return jax.nn.softmax(x, axis=axis)
def _gelu(x):
    return jax.nn.gelu(x, approximate=True)
def _silu(x):
    return jax.nn.silu(x)
def _sigmoid(x):
    return jax.nn.sigmoid(x)
def _layernorm(x, axis=-1, eps=1e-5):
    m = jnp.mean(x, axis=axis, keepdims=True)
    v = jnp.var(x, axis=axis, keepdims=True)
    return (x - m) / jnp.sqrt(v + eps)
def _scatter_add(tgt, idx, src, axis=0):
    return tgt.at[idx].add(src)
def _segment_sum(src, seg, n):
    return jax.ops.segment_sum(src, seg, n)
class _Rng:
    def __init__(self, key):
        self._k = key
    def _next(self):
        self._k, sub = jax.random.split(self._k)
        return sub
    def normal(self, shape):
        return jax.random.normal(self._next(), shape, dtype=jnp.bfloat16)
    def randint(self, lo, hi, shape):
        return jax.random.randint(self._next(), shape, lo, hi, dtype=jnp.int32)
    def uniform(self, shape, lo=0.0, hi=1.0):
        return jax.random.uniform(self._next(), shape, jnp.bfloat16, lo, hi)
    def permutation(self, n):
        return jax.random.permutation(self._next(), n)


kernel_name = 'concat_heads__gqa_block_cached__gqa_block_cached__near_ridge'

def setup_inputs():
    _rng = _Rng(jax.random.key(int.from_bytes(__import__("os").urandom(4), "little")))
    _w = (lambda a: (lambda t: t.astype(jnp.bfloat16) if jnp.issubdtype(t.dtype, jnp.floating) else t)(jnp.asarray(a)))
    def _A_setup():
        B, Sq, D = 8, 240, 640
        Hq, Hkv, Sk, Dh = 32, 32, 1024, 192
        assert Hq % Hkv == 0, (Hq, Hkv)
        return {
            "x": _w((lambda *s: _rng.normal(s) * 0.8)(B, Sq, D)),
            "k_cache": _w((lambda *s: _rng.normal(s) * 0.8)(B, Hkv, Sk, Dh)),
            "v_cache": _w((lambda *s: _rng.normal(s) * 0.05)(B, Hkv, Sk, Dh)),
            "wq": _w((lambda *s: _rng.normal(s) * 0.8)(D, Hq * Dh) * (D ** -0.5)),
            "wo": _w((lambda *s: _rng.normal(s) * 0.05)(Hq * Dh, D) * ((Hq * Dh) ** -0.5)),
        }
    _A_in = _A_setup()

    def _B_setup():
        B, Sq, D = 8, 240, 640
        Hq, Hkv, Sk, Dh = 32, 32, 1024, 192
        assert Hq % Hkv == 0, (Hq, Hkv)
        return {
            "x": _w((lambda *s: _rng.normal(s) * 0.8)(B, Sq, D)),
            "k_cache": _w((lambda *s: _rng.normal(s) * 0.8)(B, Hkv, Sk, Dh)),
            "v_cache": _w((lambda *s: _rng.normal(s) * 0.05)(B, Hkv, Sk, Dh)),
            "wq": _w((lambda *s: _rng.normal(s) * 0.8)(D, Hq * Dh) * (D ** -0.5)),
            "wo": _w((lambda *s: _rng.normal(s) * 0.05)(Hq * Dh, D) * ((Hq * Dh) ** -0.5)),
        }
    _B_in = _B_setup()

    return {
        "A_x": _A_in["x"],
        "A_k_cache": _A_in["k_cache"],
        "A_v_cache": _A_in["v_cache"],
        "A_wq": _A_in["wq"],
        "A_wo": _A_in["wo"],
        "B_x": _B_in["x"],
        "B_k_cache": _B_in["k_cache"],
        "B_v_cache": _B_in["v_cache"],
        "B_wq": _B_in["wq"],
        "B_wo": _B_in["wo"],
    }

def reference(A_x, A_k_cache, A_v_cache, A_wq, A_wo, B_x, B_k_cache, B_v_cache, B_wq, B_wo):
    def _A_ref(x, k_cache, v_cache, wq, wo):
        B, Sq, D = x.shape
        Hq, Dh = 32, 192
        Hkv = k_cache.shape[1]
        rep = Hq // Hkv
        q = (lambda x, *d: x.transpose(*d))((x @ wq).reshape(B, Sq, Hq, Dh), 0, 2, 1, 3)
        k = jnp.repeat(k_cache, rep, axis=1)
        v = jnp.repeat(v_cache, rep, axis=1)
        scores = jnp.einsum("bhqd,bhkd->bhqk", q, k) * (Dh ** -0.5)
        p = _softmax(scores, axis=-1)
        o = jnp.einsum("bhqk,bhkd->bhqd", p, v)
        return (lambda x, *d: x.transpose(*d))(o, 0, 2, 1, 3).reshape(B, Sq, Hq * Dh) @ wo

    def _B_ref(x, k_cache, v_cache, wq, wo):
        B, Sq, D = x.shape
        Hq, Dh = 32, 192
        Hkv = k_cache.shape[1]
        rep = Hq // Hkv
        q = (lambda x, *d: x.transpose(*d))((x @ wq).reshape(B, Sq, Hq, Dh), 0, 2, 1, 3)
        k = jnp.repeat(k_cache, rep, axis=1)
        v = jnp.repeat(v_cache, rep, axis=1)
        scores = jnp.einsum("bhqd,bhkd->bhqk", q, k) * (Dh ** -0.5)
        p = _softmax(scores, axis=-1)
        o = jnp.einsum("bhqk,bhkd->bhqd", p, v)
        return (lambda x, *d: x.transpose(*d))(o, 0, 2, 1, 3).reshape(B, Sq, Hq * Dh) @ wo

    a = _A_ref(A_x, A_k_cache, A_v_cache, A_wq, A_wo)
    b = _B_ref(B_x, B_k_cache, B_v_cache, B_wq, B_wo)
    return jnp.concatenate([a, b], axis=-1)
```

```python
import functools

import jax
import jax.numpy as jnp
import jax.experimental.pallas as pl
import jax.experimental.pallas.tpu as pltpu

HQ = 32
DH = 192
HPS = 2


def _kernel(ax, ak, av, awq, awo, bx, bk, bv, bwq, bwo, o_ref, acc_ref, *, d_model):
    h = pl.program_id(1)
    nh = pl.num_programs(1)
    scale = DH ** -0.5
    w = HPS * DH

    @pl.when(h == 0)
    def _():
        acc_ref[...] = jnp.zeros_like(acc_ref)

    off = pl.multiple_of(h * w, 128)
    for br, (x, k, v, wq, wo) in enumerate(((ax, ak, av, awq, awo), (bx, bk, bv, bwq, bwo))):
        qp = jnp.dot(x[0], wq[:, pl.ds(off, w)], preferred_element_type=jnp.float32)
        qp = (qp * scale).astype(jnp.bfloat16)
        outs = []
        for i in range(HPS):
            q = qp[:, i * DH:(i + 1) * DH]
            s = jnp.dot(q, k[0, i], preferred_element_type=jnp.float32)
            m = jnp.max(s, axis=-1, keepdims=True)
            p = jnp.exp(s - m)
            l = jnp.sum(p, axis=-1, keepdims=True)
            o = jax.lax.dot_general(p.astype(jnp.bfloat16), v[0, i], (((1,), (1,)), ((), ())),
                                    preferred_element_type=jnp.float32)
            outs.append((o / l).astype(jnp.bfloat16))
        oc = jnp.concatenate(outs, axis=-1)
        acc_ref[:, br * d_model:(br + 1) * d_model] += jnp.dot(
            oc, wo[pl.ds(off, w), :], preferred_element_type=jnp.float32)

    @pl.when(h == nh - 1)
    def _():
        o_ref[0] = acc_ref[...].astype(o_ref.dtype)


@jax.jit
def pallas_concat_heads__gqa_block_cached__gqa_block_cached__near_ridge_kernel(
    A_x: jax.Array,
    A_k_cache: jax.Array,
    A_v_cache: jax.Array,
    A_wq: jax.Array,
    A_wo: jax.Array,
    B_x: jax.Array,
    B_k_cache: jax.Array,
    B_v_cache: jax.Array,
    B_wq: jax.Array,
    B_wo: jax.Array,
):
    B, Sq, D = A_x.shape
    _, Hkv, Sk, Dh = A_k_cache.shape
    assert Hkv == HQ and Dh == DH

    x_spec = pl.BlockSpec((1, Sq, D), lambda b, h: (b, 0, 0))
    kv_spec = pl.BlockSpec((1, HPS, Dh, Sk), lambda b, h: (b, h, 0, 0))
    wq_spec = pl.BlockSpec((D, HQ * DH), lambda b, h: (0, 0), pipeline_mode=pl.Buffered(1))
    wo_spec = pl.BlockSpec((HQ * DH, D), lambda b, h: (0, 0), pipeline_mode=pl.Buffered(1))
    specs = [x_spec, kv_spec, kv_spec, wq_spec, wo_spec]
    tr = lambda t: jnp.transpose(t, (0, 1, 3, 2))

    return pl.pallas_call(
        functools.partial(_kernel, d_model=D),
        grid=(B, HQ // HPS),
        in_specs=specs + specs,
        out_specs=pl.BlockSpec((1, Sq, 2 * D), lambda b, h: (b, 0, 0)),
        out_shape=jax.ShapeDtypeStruct((B, Sq, 2 * D), A_x.dtype),
        scratch_shapes=[pltpu.VMEM((Sq, 2 * D), jnp.float32)],
        compiler_params=pltpu.CompilerParams(
            dimension_semantics=("arbitrary", "arbitrary"),
            vmem_limit_bytes=100 * 1024 * 1024,
        ),
    )(A_x, tr(A_k_cache), tr(A_v_cache), A_wq, A_wo, B_x, tr(B_k_cache), tr(B_v_cache), B_wq, B_wo)
```

```python
import functools

import jax
import jax.numpy as jnp
import jax.experimental.pallas as pl
import jax.experimental.pallas.tpu as pltpu

HQ = 32
DH = 192
HPS = 4


def _kernel(ax, ak, av, awq, awo, bx, bk, bv, bwq, bwo, o_ref, acc_ref, *, d_model):
    hg = pl.program_id(0)
    b = pl.program_id(1)
    nh = pl.num_programs(0)
    scale = DH ** -0.5

    branches = ((ax, ak, av, awq, awo), (bx, bk, bv, bwq, bwo))
    qps = []
    for (x, k, v, wq, wo) in branches:
        qp = jnp.dot(x[0], wq[...], preferred_element_type=jnp.float32)
        qps.append((qp * scale).astype(jnp.bfloat16))

    def qk(n):
        br, i = divmod(n, HPS)
        return jnp.dot(qps[br][:, i * DH:(i + 1) * DH], branches[br][1][0, i],
                       preferred_element_type=jnp.float32)

    s_next = qk(0)
    outs = []
    for n in range(2 * HPS):
        br, i = divmod(n, HPS)
        v, wo = branches[br][2], branches[br][4]
        s = s_next
        if n + 1 < 2 * HPS:
            s_next = qk(n + 1)
        m = jnp.max(s, axis=-1, keepdims=True)
        p = jnp.exp(s - m)
        l = jnp.sum(p, axis=-1, keepdims=True)
        p = p.astype(jnp.bfloat16)
        ot = jax.lax.dot_general(v[0, i], p, (((1,), (1,)), ((), ())),
                                 preferred_element_type=jnp.float32)
        outs.append((ot * jnp.transpose(1.0 / l)).astype(jnp.bfloat16))
        if i == HPS - 1:
            oct = jnp.concatenate(outs, axis=0)
            outs = []
            y = jax.lax.dot_general(
                oct, wo[...], (((0,), (0,)), ((), ())), preferred_element_type=jnp.float32)
            cols = slice(br * d_model, (br + 1) * d_model)
            acc_ref[b, :, cols] = jnp.where(hg == 0, 0.0, acc_ref[b, :, cols]) + y

    @pl.when(hg == nh - 1)
    def _():
        o_ref[b] = acc_ref[b].astype(o_ref.dtype)


@jax.jit
def pallas_concat_heads__gqa_block_cached__gqa_block_cached__near_ridge_kernel(
    A_x: jax.Array,
    A_k_cache: jax.Array,
    A_v_cache: jax.Array,
    A_wq: jax.Array,
    A_wo: jax.Array,
    B_x: jax.Array,
    B_k_cache: jax.Array,
    B_v_cache: jax.Array,
    B_wq: jax.Array,
    B_wo: jax.Array,
):
    B, Sq, D = A_x.shape
    _, Hkv, Sk, Dh = A_k_cache.shape
    assert Hkv == HQ and Dh == DH
    w = HPS * DH

    x_spec = pl.BlockSpec((1, Sq, D), lambda h, b: (b, 0, 0))
    kv_spec = pl.BlockSpec((1, HPS, Dh, Sk), lambda h, b: (b, h, 0, 0))
    wq_spec = pl.BlockSpec((D, w), lambda h, b: (0, h))
    wo_spec = pl.BlockSpec((w, D), lambda h, b: (h, 0))
    specs = [x_spec, kv_spec, kv_spec, wq_spec, wo_spec]
    tr = lambda t: jnp.transpose(t, (0, 1, 3, 2))

    return pl.pallas_call(
        functools.partial(_kernel, d_model=D),
        grid=(HQ // HPS, B),
        in_specs=specs + specs,
        out_specs=pl.BlockSpec((B, Sq, 2 * D), lambda h, b: (0, 0, 0)),
        out_shape=jax.ShapeDtypeStruct((B, Sq, 2 * D), A_x.dtype),
        scratch_shapes=[pltpu.VMEM((B, Sq, 2 * D), jnp.float32)],
        compiler_params=pltpu.CompilerParams(
            dimension_semantics=("arbitrary", "arbitrary"),
            vmem_limit_bytes=100 * 1024 * 1024,
        ),
    )(A_x, tr(A_k_cache), tr(A_v_cache), A_wq, A_wo, B_x, tr(B_k_cache), tr(B_v_cache), B_wq, B_wo)
```
